```python
import os as _os
_os.environ.setdefault("JAX_PLATFORMS", "cpu")
import jax
import jax.numpy as jnp

def _softmax(x, axis=-1):
    return jax.nn.softmax(x, axis=axis)
def _gelu(x):
    return jax.nn.gelu(x, approximate=True)
def _silu(x):
    return jax.nn.silu(x)
def _sigmoid(x):
    return jax.nn.sigmoid(x)
def _layernorm(x, axis=-1, eps=1e-5):
    m = jnp.mean(x, axis=axis, keepdims=True)
    v = jnp.var(x, axis=axis, keepdims=True)
    return (x - m) / jnp.sqrt(v + eps)
def _scatter_add(tgt, idx, src, axis=0):
    return tgt.at[idx].add(src)
def _segment_sum(src, seg, n):
    return jax.ops.segment_sum(src, seg, n)
class _Rng:
    def __init__(self, key):
        self._k = key
    def _next(self):
        self._k, sub = jax.random.split(self._k)
        return sub
    def normal(self, shape):
        return jax.random.normal(self._next(), shape, dtype=jnp.bfloat16)
    def randint(self, lo, hi, shape):
        return jax.random.randint(self._next(), shape, lo, hi, dtype=jnp.int32)
    def uniform(self, shape, lo=0.0, hi=1.0):
        return jax.random.uniform(self._next(), shape, jnp.bfloat16, lo, hi)
    def permutation(self, n):
        return jax.random.permutation(self._next(), n)


kernel_name = 'sequential_preLN__linear_attn_block__glu_gated_reglu__prompt'

def setup_inputs():
    _rng = _Rng(jax.random.key(int.from_bytes(__import__("os").urandom(4), "little")))
    _w = (lambda a: (lambda t: t.astype(jnp.bfloat16) if jnp.issubdtype(t.dtype, jnp.floating) else t)(jnp.asarray(a)))
    def _A_setup():
        B, S, D = 1, 2048, 640
        return {
            "x": _w((lambda *s: _rng.normal(s) * 0.05)(B, S, D)),
            "wqkv": _w((lambda *s: _rng.normal(s) * 0.05)(D, 3 * D)),
            "wo": _w((lambda *s: _rng.normal(s) * 0.05)(D, D)),
        }
    _A_in = _A_setup()

    def _B_setup():
        B, S, D, F = 1, 2048, 640, 1536
        return {
            "x": _w((lambda *s: _rng.normal(s) * 0.05)(B, S, D)),
            "W_gate": _w((lambda *s: _rng.normal(s) * 0.05)(D, F) * (2.0 / D) ** 0.5),
            "W_up": _w((lambda *s: _rng.normal(s) * 0.05)(D, F) * (2.0 / D) ** 0.5),
            "W_down": _w((lambda *s: _rng.normal(s) * 0.05)(F, D) * (1.0 / F) ** 0.5),
        }
    _B_in = _B_setup()

    return {
        "A_x": _A_in["x"],
        "A_wqkv": _A_in["wqkv"],
        "A_wo": _A_in["wo"],
        "B_x": _B_in["x"],
        "B_W_gate": _B_in["W_gate"],
        "B_W_up": _B_in["W_up"],
        "B_W_down": _B_in["W_down"],
    }

def reference(A_x, A_wqkv, A_wo, B_x, B_W_gate, B_W_up, B_W_down):
    def _A_ref(x, wqkv, wo):
        B, S, D = x.shape
        H = 32; Dh = D // H
        qkv = (lambda x, *d: x.transpose(*d))((x @ wqkv).reshape(B, S, 3, H, Dh), 2, 0, 3, 1, 4)
        q, k, v = qkv[0], qkv[1], qkv[2]
        phi = lambda t: jnp.where(t > 0, t + 1, jnp.exp(t)) + 1e-6
        pq, pk = phi(q), phi(k)
        kv = jnp.einsum("bhsd,bhse->bhde", pk, v)
        z = jnp.einsum("bhsd->bhd", pk)
        num = jnp.einsum("bhqd,bhde->bhqe", pq, kv)
        den = jnp.einsum("bhqd,bhd->bhq", pq, z)[..., None] + 1e-6
        o = num / den
        return (lambda x, *d: x.transpose(*d))(o, 0, 2, 1, 3).reshape(B, S, D) @ wo

    def _B_ref(x, W_gate, W_up, W_down):
        gate = jnp.einsum("bsd,df->bsf", x, W_gate)
        up = jnp.einsum("bsd,df->bsf", x, W_up)
        gate = gate * (lambda x, dt: x.astype(dt))(gate > 0, gate.dtype)
        h = gate * up
        return jnp.einsum("bsf,fd->bsd", h, W_down)

    x = A_x
    h = x + _A_ref(_layernorm(x, axis=-1), A_wqkv, A_wo)
    h2 = h + _B_ref(_layernorm(h, axis=-1), B_W_gate, B_W_up, B_W_down)
    return h2
```

```python
import jax
import jax.numpy as jnp
from jax import lax
import jax.experimental.pallas as pl
import jax.experimental.pallas.tpu as pltpu

S, D, F, H = 2048, 640, 1536, 32
DH = D // H
T = 256
FC = 512
LC = 64
NT = S // T
F32, BF16 = jnp.float32, jnp.bfloat16
BANDS = [(16 * ((128 * j // DH) * DH // 16), min(D, -16 * (-(((128 * j + 127) // DH + 1) * DH) // 16)))
         for j in range(D // 128)]


def _ln(x):
    m = jnp.mean(x, axis=-1, keepdims=True)
    c = x - m
    v = jnp.mean(c * c, axis=-1, keepdims=True)
    return c * lax.rsqrt(v + 1e-5)


def _phi(t):
    return jnp.where(t > 0, t + 1.0, jnp.exp(t)) + 1e-6


def _mm(a, b):
    return jnp.dot(a, b, preferred_element_type=F32)


def _kernel(x_hbm, wqkv_hbm, wo_hbm, wg_hbm, wu_hbm, wd_hbm, out_hbm,
            x_v, xn_v, wq_v, wk_v, wv_v, wo_v, wg_v, wu_v, wd_v, g_v, macc_v, m_v, zt_v, zp_v, zrow_v, wqt_v, wqp_v, o_v, xp_v, pkt_v, h_v, hn_v,
            x_sem, w_sem, o_sem):
    def rows(i):
        return pl.ds(pl.multiple_of(i * T, T), T)

    def x_copy(i):
        return pltpu.make_async_copy(x_hbm.at[rows(i), :], x_v.at[rows(i), :], x_sem.at[i])

    def o_copy(i):
        return pltpu.make_async_copy(o_v.at[rows(i), :], out_hbm.at[rows(i), :], o_sem.at[i])

    cp_wk = pltpu.make_async_copy(wqkv_hbm.at[:, pl.ds(D, D)], wk_v, w_sem.at[0])
    cp_wv = pltpu.make_async_copy(wqkv_hbm.at[:, pl.ds(2 * D, D)], wv_v, w_sem.at[1])
    cp_wo = pltpu.make_async_copy(wo_hbm, wo_v, w_sem.at[2])
    cp_wq = pltpu.make_async_copy(wqkv_hbm.at[:, pl.ds(0, D)], wq_v, w_sem.at[3])
    cp_wg = pltpu.make_async_copy(wg_hbm, wg_v, w_sem.at[4])
    cp_wu = pltpu.make_async_copy(wu_hbm, wu_v, w_sem.at[5])
    cp_wd = pltpu.make_async_copy(wd_hbm, wd_v, w_sem.at[6])

    x_copy(0).start()
    cp_wk.start()
    g_v[...] = jnp.zeros_like(g_v)
    x_copy(0).wait()
    for i in range(1, NT):
        x_copy(i).start()

    def ln_k(i, slot, first=False):
        for r0 in range(0, T, LC):
            xr = x_v[pl.ds(pl.multiple_of(i * T + r0, LC), LC), :]
            xp_v[r0:r0 + LC, :] = _ln(xr.astype(F32)).astype(BF16)
        if first:
            cp_wk.wait()
            for c in (cp_wv, cp_wo, cp_wq, cp_wg, cp_wu, cp_wd):
                c.start()
        pk = _phi(_mm(xp_v[...], wk_v[...])).astype(BF16)
        pkt_v[slot] = pk.T
        return jnp.sum(pk.astype(F32).reshape(T // 8, 8, D), axis=0)

    def g_part(i, slot, c0, c1):
        g_v[:, c0:c1] += _mm(pkt_v[slot], xn_v[rows(i), c0:c1])

    zacc = ln_k(0, 0, True)
    xn_v[rows(0), :] = xp_v[...]

    def p1_tile(i, u, zacc):
        g_part(i - 1, u, 0, 384)
        zacc = zacc + ln_k(i, 1 - u)
        g_part(i - 1, u, 384, D)
        xn_v[rows(i), :] = xp_v[...]
        return zacc

    def p1(j, zacc):
        x_copy(2 * j + 1).wait()
        x_copy(2 * j + 2).wait()
        zacc = p1_tile(2 * j + 1, 0, zacc)
        return p1_tile(2 * j + 2, 1, zacc)

    zacc = lax.fori_loop(0, NT // 2 - 1, p1, zacc)
    x_copy(NT - 1).wait()
    cp_wv.wait()
    cp_wo.wait()
    cp_wq.wait()
    zacc = p1_tile(NT - 1, 0, zacc)
    g_part(NT - 1, 1, 0, D)
    z = jnp.sum(zacc, axis=0, keepdims=True)

    macc_v[...] = jnp.zeros_like(macc_v)
    NC = D // 128
    for j, (r0, r1) in enumerate(BANDS):
        cs = slice(128 * j, 128 * (j + 1))
        kv = _mm(g_v[r0:r1, :].astype(BF16), wv_v[:, cs])
        rh = (lax.broadcasted_iota(jnp.int32, (r1 - r0, 128), 0) + r0) // DH
        ch = (lax.broadcasted_iota(jnp.int32, (r1 - r0, 128), 1) + 128 * j) // DH
        kv = jnp.where(rh == ch, kv, 0.0).astype(BF16)
        mj = _mm(kv, wo_v[cs, :])
        for t in range(NC):
            macc_v[t, r0:r1, :] += mj[:, 128 * t:128 * (t + 1)]
    zt_v[...] = jnp.transpose(jnp.broadcast_to(z, (128, D)))
    for t in range(NC):
        wqt_v[t] = jnp.transpose(wq_v[128 * t:128 * (t + 1), :].astype(F32))
    for j in range(DH):
        src, dst = pl.ds(j, H, stride=DH), slice(j * H, (j + 1) * H)
        for t in range(NC):
            m_v[dst, 128 * t:128 * (t + 1)] = macc_v[t, src, :].astype(BF16)
            wqp_v[dst, 128 * t:128 * (t + 1)] = wqt_v[t, src, :].astype(BF16)
        zp_v[dst, :] = zt_v[src, :]
    zrow_v[...] = jnp.transpose(zp_v[...])[0:8, :]

    def attn_a(i):
        q = lax.dot_general(xn_v[rows(i), :], wqp_v[...], (((1,), (1,)), ((), ())), preferred_element_type=F32)
        pq = _phi(q)
        t = (pq.reshape(T // 8, 8, D) * zrow_v[...][None]).reshape(T, D)
        den = t[:, 0:128] + t[:, 128:256] + t[:, 256:384] + t[:, 384:512] + t[:, 512:640]
        den = den + pltpu.roll(den, 64, 1)
        den = den + pltpu.roll(den, 32, 1)
        r = 1.0 / (den + 1e-6)
        return (pq * jnp.concatenate([r] * (D // 128), axis=1)).astype(BF16)

    def attn_b(i, pqs):
        h_v[...] = x_v[rows(i), :].astype(F32) + _mm(pqs, m_v[...])

    def ln2():
        for r0 in range(0, T, LC):
            hn_v[r0:r0 + LC, :] = _ln(h_v[r0:r0 + LC, :]).astype(BF16)

    def ffn(i, with_next):
        nc = F // FC
        acc = h_v[...]
        for c in range(nc):
            cs = slice(c * FC, (c + 1) * FC)
            gate = _mm(hn_v[...], wg_v[:, cs])
            up = _mm(hn_v[...], wu_v[:, cs])
            if with_next and c == 0:
                pqs = attn_a(i + 1)
            if with_next and c == 1:
                attn_b(i + 1, pqs)
            if with_next and c == nc - 1:
                ln2()
            act = (jnp.maximum(gate, 0.0) * up).astype(BF16)
            acc = acc + _mm(act, wd_v[cs, :])
        o_v[rows(i), :] = acc.astype(BF16)
        o_copy(i).start()

    attn_b(0, attn_a(0))
    ln2()
    cp_wg.wait()
    cp_wu.wait()
    cp_wd.wait()

    def p2(i, carry):
        ffn(i, True)
        return carry

    lax.fori_loop(0, NT - 1, p2, 0)
    ffn(NT - 1, False)
    for i in range(NT):
        o_copy(i).wait()


@jax.jit
def pallas_sequential_preLN__linear_attn_block__glu_gated_reglu__prompt_kernel(
        A_x, A_wqkv, A_wo, B_x, B_W_gate, B_W_up, B_W_down):
    x2 = A_x.reshape(S, D)
    any_spec = pl.BlockSpec(memory_space=pl.ANY)
    out = pl.pallas_call(
        _kernel,
        out_shape=jax.ShapeDtypeStruct((S, D), BF16),
        in_specs=[any_spec] * 6,
        out_specs=any_spec,
        scratch_shapes=[
            pltpu.VMEM((S, D), BF16),
            pltpu.VMEM((S, D), BF16),
            pltpu.VMEM((D, D), BF16),
            pltpu.VMEM((D, D), BF16),
            pltpu.VMEM((D, D), BF16),
            pltpu.VMEM((D, D), BF16),
            pltpu.VMEM((D, F), BF16),
            pltpu.VMEM((D, F), BF16),
            pltpu.VMEM((F, D), BF16),
            pltpu.VMEM((D, D), F32),
            pltpu.VMEM((D // 128, D, 128), F32),
            pltpu.VMEM((D, D), BF16),
            pltpu.VMEM((D, 128), F32),
            pltpu.VMEM((D, 128), F32),
            pltpu.VMEM((8, D), F32),
            pltpu.VMEM((D // 128, D, 128), F32),
            pltpu.VMEM((D, D), BF16),
            pltpu.VMEM((S, D), BF16),
            pltpu.VMEM((T, D), BF16),
            pltpu.VMEM((2, D, T), BF16),
            pltpu.VMEM((T, D), F32),
            pltpu.VMEM((T, D), BF16),
            pltpu.SemaphoreType.DMA((NT,)),
            pltpu.SemaphoreType.DMA((7,)),
            pltpu.SemaphoreType.DMA((NT,)),
        ],
        compiler_params=pltpu.CompilerParams(vmem_limit_bytes=100 * 1024 * 1024),
    )(x2, A_wqkv, A_wo, B_W_gate, B_W_up, B_W_down)
    return out.reshape(1, S, D)
```

```python
import jax
import jax.numpy as jnp
from jax import lax
import jax.experimental.pallas as pl
import jax.experimental.pallas.tpu as pltpu

S, D, F, H = 2048, 640, 1536, 32
DH = D // H
T = 256
FCS = (512, 512, 512)
PA, PB, PL = 0, 2, 2
GS = 384
LC = 64
NT = S // T
F32, BF16 = jnp.float32, jnp.bfloat16
BANDS = [(16 * ((128 * j // DH) * DH // 16), min(D, -16 * (-(((128 * j + 127) // DH + 1) * DH) // 16)))
         for j in range(D // 128)]


def _ln(x):
    m = jnp.mean(x, axis=-1, keepdims=True)
    c = x - m
    v = jnp.mean(c * c, axis=-1, keepdims=True)
    return c * lax.rsqrt(v + 1e-5)


def _phi(t):
    return jnp.where(t > 0, t + 1.0, jnp.exp(t)) + 1e-6


def _mm(a, b):
    return jnp.dot(a, b, preferred_element_type=F32)


def _kernel(x_hbm, wqkv_hbm, wo_hbm, wg_hbm, wu_hbm, wd_hbm, out_hbm,
            x_v, xn_v, wq_v, wk_v, wv_v, wo_v, wg_v, wu_v, wd_v, g_v, macc_v, m_v, zt_v, zp_v, zrow_v, wqt_v, wqp_v, o_v, xp_v, pkt_v, h_v, hn_v,
            x_sem, w_sem, o_sem):
    def rows(i):
        return pl.ds(pl.multiple_of(i * T, T), T)

    def x_copy(i):
        return pltpu.make_async_copy(x_hbm.at[rows(i), :], x_v.at[rows(i), :], x_sem.at[i])

    def o_copy(i):
        return pltpu.make_async_copy(o_v.at[rows(i), :], out_hbm.at[rows(i), :], o_sem.at[i])

    def last_copy(hf):
        rs = pl.ds((NT - 1) * T + hf * (T // 2), T // 2)
        return pltpu.make_async_copy(o_v.at[rs, :], out_hbm.at[rs, :], o_sem.at[NT - 1 + hf])

    cp_wk = pltpu.make_async_copy(wqkv_hbm.at[:, pl.ds(D, D)], wk_v, w_sem.at[0])
    cp_wv = pltpu.make_async_copy(wqkv_hbm.at[:, pl.ds(2 * D, D)], wv_v, w_sem.at[1])
    cp_wo = pltpu.make_async_copy(wo_hbm, wo_v, w_sem.at[2])
    cp_wq = pltpu.make_async_copy(wqkv_hbm.at[:, pl.ds(0, D)], wq_v, w_sem.at[3])
    cp_wg = pltpu.make_async_copy(wg_hbm, wg_v, w_sem.at[4])
    cp_wu = pltpu.make_async_copy(wu_hbm, wu_v, w_sem.at[5])
    cp_wd = pltpu.make_async_copy(wd_hbm, wd_v, w_sem.at[6])

    x_copy(0).start()
    cp_wk.start()
    g_v[...] = jnp.zeros_like(g_v)
    x_copy(0).wait()

    def ln_k(i, slot, first=False):
        for r0 in range(0, T, LC):
            xr = x_v[pl.ds(pl.multiple_of(i * T + r0, LC), LC), :]
            xp_v[r0:r0 + LC, :] = _ln(xr.astype(F32)).astype(BF16)
        if first:
            cp_wk.wait()
            for n in range(1, NT):
                x_copy(n).start()
            for c in (cp_wv, cp_wo, cp_wq, cp_wg, cp_wu, cp_wd):
                c.start()
        pk = _phi(_mm(xp_v[...], wk_v[...])).astype(BF16)
        pkt_v[slot] = pk.T
        return jnp.sum(pk.astype(F32).reshape(T // 8, 8, D), axis=0)

    def g_part(i, slot, c0, c1):
        g_v[:, c0:c1] += _mm(pkt_v[slot], xn_v[rows(i), c0:c1])

    zacc = ln_k(0, 0, True)
    xn_v[rows(0), :] = xp_v[...]

    def p1_tile(i, u, zacc):
        g_part(i - 1, u, 0, GS)
        zacc = zacc + ln_k(i, 1 - u)
        g_part(i - 1, u, GS, D)
        xn_v[rows(i), :] = xp_v[...]
        return zacc

    def p1(j, zacc):
        x_copy(2 * j + 1).wait()
        x_copy(2 * j + 2).wait()
        zacc = p1_tile(2 * j + 1, 0, zacc)
        return p1_tile(2 * j + 2, 1, zacc)

    zacc = lax.fori_loop(0, NT // 2 - 1, p1, zacc)
    x_copy(NT - 1).wait()
    cp_wv.wait()
    cp_wo.wait()
    cp_wq.wait()
    NC = D // 128
    for t in range(NC):
        wqt_v[t] = jnp.transpose(wq_v[128 * t:128 * (t + 1), :].astype(F32))
    for j in range(DH):
        for t in range(NC):
            wqp_v[j * H:(j + 1) * H, 128 * t:128 * (t + 1)] = wqt_v[t, pl.ds(j, H, stride=DH), :].astype(BF16)
    zacc = p1_tile(NT - 1, 0, zacc)
    g_part(NT - 1, 1, 0, D)
    z = jnp.sum(zacc, axis=0, keepdims=True)

    def attn_q(i):
        q = lax.dot_general(xn_v[rows(i), :], wqp_v[...], (((1,), (1,)), ((), ())), preferred_element_type=F32)
        return _phi(q)

    pq0 = attn_q(0)

    macc_v[...] = jnp.zeros_like(macc_v)
    for j, (r0, r1) in enumerate(BANDS):
        cs = slice(128 * j, 128 * (j + 1))
        kv = _mm(g_v[r0:r1, :].astype(BF16), wv_v[:, cs])
        rh = (lax.broadcasted_iota(jnp.int32, (r1 - r0, 128), 0) + r0) // DH
        ch = (lax.broadcasted_iota(jnp.int32, (r1 - r0, 128), 1) + 128 * j) // DH
        kv = jnp.where(rh == ch, kv, 0.0).astype(BF16)
        mj = _mm(kv, wo_v[cs, :])
        for t in range(NC):
            macc_v[t, r0:r1, :] += mj[:, 128 * t:128 * (t + 1)]
    zt_v[...] = jnp.transpose(jnp.broadcast_to(z, (128, D)))
    for j in range(DH):
        src, dst = pl.ds(j, H, stride=DH), slice(j * H, (j + 1) * H)
        for t in range(NC):
            m_v[dst, 128 * t:128 * (t + 1)] = macc_v[t, src, :].astype(BF16)
        zp_v[dst, :] = zt_v[src, :]
    zrow_v[...] = jnp.transpose(zp_v[...])[0:8, :]

    def attn_d(pq):
        t = (pq.reshape(T // 8, 8, D) * zrow_v[...][None]).reshape(T, D)
        den = t[:, 0:128] + t[:, 128:256] + t[:, 256:384] + t[:, 384:512] + t[:, 512:640]
        den = den + pltpu.roll(den, 64, 1)
        den = den + pltpu.roll(den, 32, 1)
        r = 1.0 / (den + 1e-6)
        return (pq * jnp.concatenate([r] * (D // 128), axis=1)).astype(BF16)

    def attn_b(i, pqs):
        h_v[...] = x_v[rows(i), :].astype(F32) + _mm(pqs, m_v[...])

    def ln2():
        for r0 in range(0, T, LC):
            hn_v[r0:r0 + LC, :] = _ln(h_v[r0:r0 + LC, :]).astype(BF16)

    def ffn(i, with_next):
        nc = len(FCS)
        acc = h_v[...]
        for c in range(nc):
            cs = slice(sum(FCS[:c]), sum(FCS[:c + 1]))
            gate = _mm(hn_v[...], wg_v[:, cs])
            up = _mm(hn_v[...], wu_v[:, cs])
            if with_next and c == PA:
                pqs = attn_d(attn_q(i + 1))
            if with_next and c == PB:
                attn_b(i + 1, pqs)
            if with_next and c == PL:
                ln2()
            act = (jnp.maximum(gate, 0.0) * up).astype(BF16)
            if not with_next and c == nc - 1:
                for hf in range(2):
                    r0 = i * T + hf * (T // 2)
                    rs = slice(hf * (T // 2), (hf + 1) * (T // 2))
                    o_v[r0:r0 + T // 2, :] = (acc[rs] + _mm(act[rs], wd_v[cs, :])).astype(BF16)
                    last_copy(hf).start()
                return
            acc = acc + _mm(act, wd_v[cs, :])
        o_v[rows(i), :] = acc.astype(BF16)
        o_copy(i).start()

    attn_b(0, attn_d(pq0))
    ln2()
    cp_wg.wait()
    cp_wu.wait()
    cp_wd.wait()

    def p2(i, carry):
        ffn(i, True)
        return carry

    lax.fori_loop(0, NT - 1, p2, 0)
    ffn(NT - 1, False)
    for i in range(NT - 1):
        o_copy(i).wait()
    last_copy(0).wait()
    last_copy(1).wait()


@jax.jit
def pallas_sequential_preLN__linear_attn_block__glu_gated_reglu__prompt_kernel(
        A_x, A_wqkv, A_wo, B_x, B_W_gate, B_W_up, B_W_down):
    x2 = A_x.reshape(S, D)
    any_spec = pl.BlockSpec(memory_space=pl.ANY)
    out = pl.pallas_call(
        _kernel,
        out_shape=jax.ShapeDtypeStruct((S, D), BF16),
        in_specs=[any_spec] * 6,
        out_specs=any_spec,
        scratch_shapes=[
            pltpu.VMEM((S, D), BF16),
            pltpu.VMEM((S, D), BF16),
            pltpu.VMEM((D, D), BF16),
            pltpu.VMEM((D, D), BF16),
            pltpu.VMEM((D, D), BF16),
            pltpu.VMEM((D, D), BF16),
            pltpu.VMEM((D, F), BF16),
            pltpu.VMEM((D, F), BF16),
            pltpu.VMEM((F, D), BF16),
            pltpu.VMEM((D, D), F32),
            pltpu.VMEM((D // 128, D, 128), F32),
            pltpu.VMEM((D, D), BF16),
            pltpu.VMEM((D, 128), F32),
            pltpu.VMEM((D, 128), F32),
            pltpu.VMEM((8, D), F32),
            pltpu.VMEM((D // 128, D, 128), F32),
            pltpu.VMEM((D, D), BF16),
            pltpu.VMEM((S, D), BF16),
            pltpu.VMEM((T, D), BF16),
            pltpu.VMEM((2, D, T), BF16),
            pltpu.VMEM((T, D), F32),
            pltpu.VMEM((T, D), BF16),
            pltpu.SemaphoreType.DMA((NT,)),
            pltpu.SemaphoreType.DMA((7,)),
            pltpu.SemaphoreType.DMA((NT + 1,)),
        ],
        compiler_params=pltpu.CompilerParams(vmem_limit_bytes=100 * 1024 * 1024),
    )(x2, A_wqkv, A_wo, B_W_gate, B_W_up, B_W_down)
    return out.reshape(1, S, D)
```
